```python
import os as _os
_os.environ.setdefault('JAX_PLATFORMS', 'cpu')
import jax
import jax.numpy as jnp

def _softmax(x, axis=-1):
    return jax.nn.softmax(x, axis=axis)

def _gelu(x):
    return jax.nn.gelu(x, approximate=True)

def _silu(x):
    return jax.nn.silu(x)

def _sigmoid(x):
    return jax.nn.sigmoid(x)

def _layernorm(x, axis=-1, eps=1e-05):
    m = jnp.mean(x, axis=axis, keepdims=True)
    v = jnp.var(x, axis=axis, keepdims=True)
    return (x - m) / jnp.sqrt(v + eps)

def _scatter_add(tgt, idx, src, axis=0):
    return tgt.at[idx].add(src)

def _segment_sum(src, seg, n):
    return jax.ops.segment_sum(src, seg, n)

class _Rng:

    def __init__(self, key):
        self._k = key

    def _next(self):
        self._k, sub = jax.random.split(self._k)
        return sub

    def normal(self, shape):
        return jax.random.normal(self._next(), shape, dtype=jnp.bfloat16)

    def randint(self, lo, hi, shape):
        return jax.random.randint(self._next(), shape, lo, hi, dtype=jnp.int32)

    def uniform(self, shape, lo=0.0, hi=1.0):
        return jax.random.uniform(self._next(), shape, jnp.bfloat16, lo, hi)

    def permutation(self, n):
        return jax.random.permutation(self._next(), n)
kernel_name = 'adaLN_cond__ssm_conv_h3__moe_arch_mod__prompt'

def setup_inputs():
    _rng = _Rng(jax.random.key(int.from_bytes(__import__("os").urandom(4), "little")))
    _w = lambda a: (lambda t: t.astype(jnp.bfloat16) if jnp.issubdtype(t.dtype, jnp.floating) else t)(jnp.asarray(a))

    def _A_setup():
        B, S, D = (1, 2048, 640)
        ks = 4
        return {'q': _w((lambda *s: _rng.normal(s) * 0.05)(B, S, D)), 'k': _w((lambda *s: _rng.normal(s) * 0.4)(B, S, D)), 'v': _w((lambda *s: _rng.normal(s) * 0.4)(B, S, D)), 'shift_k': _w((lambda *s: _rng.normal(s) * 0.4)(D, ks) * 0.5), 'ssm_k': _w((lambda *s: _rng.normal(s) * 0.4)(D, S) * (1.0 / S ** 0.5)), 'ssm_D': _w((lambda *s: _rng.normal(s) * 0.4)(D))}
    _A_in = _A_setup()

    def _B_setup():
        B, S, D, F, C = (1, 2048, 640, 1728, 2)
        return {'x': _w((lambda *s: _rng.normal(s) * 0.05)(B, S, D)), 'w_r': _w((lambda *s: _rng.normal(s) * 0.1)(D)), 'w_gate': _w((lambda *s: _rng.normal(s) * 0.1)(D, F)), 'w_up': _w((lambda *s: _rng.normal(s) * 0.1)(D, F)), 'w_down': _w((lambda *s: _rng.normal(s) * 0.1)(F, D))}
    _B_in = _B_setup()
    return {'A_q': _A_in['q'], 'A_k': _A_in['k'], 'A_v': _A_in['v'], 'A_shift_k': _A_in['shift_k'], 'A_ssm_k': _A_in['ssm_k'], 'A_ssm_D': _A_in['ssm_D'], 'B_x': _B_in['x'], 'B_w_r': _B_in['w_r'], 'B_w_gate': _B_in['w_gate'], 'B_w_up': _B_in['w_up'], 'B_w_down': _B_in['w_down'], 'c': _w((lambda *s: _rng.normal(s) * 0.2)(1, 640) * 8.0), 'w_mod': _w((lambda *s: _rng.normal(s) * 0.2)(640, 6 * 640) * 640 ** (-0.5) * 8.0)}

def reference(A_q, A_k, A_v, A_shift_k, A_ssm_k, A_ssm_D, B_x, B_w_r, B_w_gate, B_w_up, B_w_down, c, w_mod):

    def _A_ref(q, k, v, shift_k, ssm_k, ssm_D):
        B, S, D = q.shape
        ks = shift_k.shape[-1]
        k_pad = jnp.pad(k, ((0, 0), (ks - 1, 0), (0, 0)))
        k_shift = jnp.zeros_like(k)
        for t in range(ks):
            k_shift = k_shift + k_pad[:, t:t + S, :] * shift_k[:, ks - 1 - t][None, None, :]
        kv = k_shift * v
        L = 2 * S
        kv_pad = jnp.pad(kv, ((0, 0), (0, S), (0, 0)))
        kf_pad = jnp.pad(ssm_k, ((0, 0), (0, S)))
        kv_f = (lambda x, axes=(-2, -1): jnp.fft.rfft2(x.astype(jnp.float32), axes=axes))(kv_pad[:, None, :, :], axes=(1, 2))
        kf_f = (lambda x, axes=(-2, -1): jnp.fft.rfft2(x.astype(jnp.float32), axes=axes))(kf_pad[:, None, :], axes=(1, 2))
        kf_f = (lambda x, *d: x.transpose(*d))(kf_f, 1, 2, 0)
        y_f = kv_f * kf_f[None, :, :, :]
        y = (lambda x, s, axes=(-2, -1): jnp.fft.irfft2(x, s=s, axes=axes).astype(jnp.bfloat16))(y_f, (1, L), axes=(1, 2))[:, 0, :S, :]
        y = y + kv * ssm_D[None, None, :]
        return q * y

    def _B_ref(x, w_r, w_gate, w_up, w_down):
        B, S, D = x.shape
        C = 2
        r = x @ w_r
        idx = jnp.argsort(-r, axis=-1)[:, :C]
        idx_e = jnp.repeat(idx.reshape(B, C, 1), D, axis=2)
        x_sel = jnp.take_along_axis(x, idx_e, axis=1)
        g = _silu(x_sel @ w_gate)
        u = x_sel @ w_up
        y = g * u @ w_down
        r_sel = _sigmoid(jnp.take_along_axis(r, idx, axis=1))
        y = y * r_sel.reshape(B, C, 1)
        b_off = (jnp.arange(B) * S).reshape(B, 1)
        flat_idx = (idx + b_off).reshape(B * C)
        zero = (x * 0.0).reshape(B * S, D)
        upd = _scatter_add(zero, flat_idx, y.reshape(B * C, D), axis=0)
        return x + upd.reshape(B, S, D)
    x = A_q
    mod = (_silu(c) @ w_mod).reshape(c.shape[0], 6, 1, -1)
    sa, ca, ga, sb, cb, gb = (mod[:, 0].copy(), mod[:, 1].copy(), mod[:, 2].copy(), mod[:, 3].copy(), mod[:, 4].copy(), mod[:, 5].copy())
    h = _layernorm(x, axis=-1) * (1 + ca) + sa
    x = x + ga * _A_ref(h, A_k, A_v, A_shift_k, A_ssm_k, A_ssm_D)
    h = _layernorm(x, axis=-1) * (1 + cb) + sb
    x = x + gb * _B_ref(h, B_w_r, B_w_gate, B_w_up, B_w_down)
    return x
```

```python
import os
import numpy as np
import jax
import jax.numpy as jnp
from jax import lax
import jax.experimental.pallas as pl
import jax.experimental.pallas.tpu as pltpu

S, D, FF = 2048, 640, 1728
BLK = 128
NB = S // BLK
NT = D // 128
EPS = 1e-5
F32, BF16, U32 = jnp.float32, jnp.bfloat16, jnp.uint32
FCH = ((0, 512), (512, 512), (1024, 384), (1408, 192), (1600, 128))
GROUPS = tuple(int(x) for x in os.environ.get('GROUPS_', '4,4,4,4').split(','))
UB = int(os.environ.get('UB', 2))
NI = NB // UB
RG = int(os.environ.get('RG', 64))
NG = S // RG
SL = int(os.environ.get('SL', 16))
SCOPES = False


def _bf16_bits(a):
    u = np.ascontiguousarray(a, np.float32).view(np.uint32)
    return ((u + 0x7FFF + ((u >> 16) & 1)) >> 16).astype(np.uint32)


def _pack_rows(a):
    b = _bf16_bits(a)
    return (b[0::2] | (b[1::2] << 16)).astype(np.uint32)


def _dft_mats():
    m = np.arange(128)[:, None]
    s = np.arange(128)[None, :]
    ang = np.pi * (((4 * m + 1) * s) % 512) / 256.0
    c, sn = np.cos(ang), np.sin(ang)
    fwd = np.stack([c.reshape(16, 8, 128), (-sn).reshape(16, 8, 128)], axis=1).reshape(256, 128)
    inv = fwd.T / 128.0
    return _pack_rows(fwd), np.stack([_pack_rows(inv[:, :128]), _pack_rows(inv[:, 128:])])


def _nt(a, b):
    return lax.dot_general(a, b, (((1,), (1,)), ((), ())), preferred_element_type=F32)


def _nn(a, b):
    return jnp.dot(a, b, preferred_element_type=F32)


def _bf(x):
    return pltpu.bitcast(x, BF16)


class _NoScope:
    def __enter__(self):
        return self

    def __exit__(self, *a):
        return False


def _scope(name):
    return jax.named_scope(name) if SCOPES else _NoScope()


def _kernel(q_h, k_h, v_h, sk_h, ssm_h, dd_h, wr_h, wg_h, wu_h, wd_h, c_h, wm_h, fw_h, iv_h,
            o_h,
            q_s, k_s, v_s, sk_s, ssm_u, dd_s, wr_s, wg_u, wu_u, wd_u, c_s, wm_u, fw_s, iv_s,
            kf_s, kv_s, tap_s, x0_s, x1_s, k0_s, k1_s, z0_s, z1_s, ya_s, yb_s, mp_s, cf_s,
            n2_s, o_s, r_s, st_s, pt_s, xx_s, cv_s, zero_s,
            sem_i, sem_o):
    xs, ks, zs = (x0_s, x1_s), (k0_s, k1_s), (z0_s, z1_s)
    zv = (z0_s.bitcast(U32), z1_s.bitcast(U32))
    kv_v = kv_s.bitcast(U32)
    n2_v = n2_s.bitcast(U32)
    ssm_s, wg_s, wu_s, wd_s, wm_s = (r.bitcast(BF16) for r in (ssm_u, wg_u, wu_u, wd_u, wm_u))

    nsem = [0]

    def mk(src, dst):
        cp = pltpu.make_async_copy(src, dst, sem_i.at[nsem[0]])
        nsem[0] += 1
        return cp

    small = [mk(a, b) for a, b in
             ((fw_h, fw_s), (sk_h, sk_s), (iv_h, iv_s), (dd_h, dd_s), (wr_h, wr_s), (c_h, c_s))]
    kv_cps, ssm_cps = [], []
    for l in range(NT):
        cols = pl.ds(l * 128, 128)
        kv_cps.append([mk(k_h.at[:, cols], k_s.at[l]), mk(v_h.at[:, cols], v_s.at[l])])
        ssm_cps.append(mk(ssm_h.at[cols, :], ssm_s.at[cols, :]))
    wm_cp = mk(wm_h, wm_s)
    q_cp = mk(q_h, q_s)
    f_cps = []
    for st, n in FCH:
        rows = pl.ds(st, n)
        f_cps.append([mk(h.at[rows], s.at[rows]) for h, s in ((wg_h, wg_s), (wu_h, wu_s), (wd_h, wd_s))])

    def o_copy(b):
        rows = pl.ds(pl.multiple_of(b * BLK, BLK), BLK)
        return pltpu.make_async_copy(o_s.at[rows], o_h.at[rows], sem_o.at[b])

    order = list(small)
    for l in range(NT):
        order += kv_cps[l] + [ssm_cps[l]]
    for cp in order + [wm_cp, q_cp] + sum(f_cps, []):
        cp.start()

    kf_s[pl.ds(0, 8), :] = jnp.zeros((8, 128), F32)
    for g in range(8):
        zero_s[g] = 0
    for cp in small:
        cp.wait()
    skf = sk_s[...].astype(F32)
    for l in range(NT):
        for j in range(4):
            tap_s[l, j] = jnp.broadcast_to(skf[j:j + 1, l * 128:(l + 1) * 128], (8, 128))
    cv = c_s[...].astype(F32)
    cv_s[...] = pltpu.bitcast(jnp.broadcast_to((cv * jax.nn.sigmoid(cv)).astype(BF16), (16, D)), U32)

    def make_kv(l, t):
        r0 = pl.multiple_of(t * BLK, BLK)
        kb = k_s[l, pl.ds(r0, BLK), :].astype(F32)
        kf_s[pl.ds(r0 + 8, BLK), :] = kb
        w = [jnp.tile(tap_s[l, j], (BLK // 8, 1)) for j in range(4)]
        acc = kb * w[0]
        for j in range(1, 4):
            acc = acc + kf_s[pl.ds(r0 + 8 - j, BLK), :] * w[j]
        kv_s[t] = (acc * v_s[l, pl.ds(r0, BLK), :].astype(F32)).astype(BF16)

    def fwd_k(l, t):
        r0 = pl.multiple_of(t * BLK, BLK)
        ks[l % 2][t] = _nt(_bf(fw_s[...]), ssm_s[l * 128:(l + 1) * 128, pl.ds(r0, BLK)]).reshape(16, 2, 8, 128)

    def fwd_x(l, t):
        xs[l % 2][t] = _nn(_bf(fw_s[...]), _bf(kv_v[t])).reshape(16, 2, 8, 128)

    def add_skip(l):
        kk_s = ks[l % 2]
        kk_s[0, :, 0] = kk_s[0, :, 0] + dd_s[l:l + 1, :].astype(F32)

    def wconv(l, t0):
        x_s, kk_s, z_s = xs[l % 2], ks[l % 2], zs[l % 2]
        zrows = pl.ds(pl.multiple_of(t0 * 16, 16), 16)
        prev = None
        b0 = 0
        for g, gs in enumerate(GROUPS):
            t = t0 + zero_s[g]
            acc = [None] * gs
            xw = {}
            for j in range(b0 + gs):
                kc, kd = kk_s[j, t, 0], kk_s[j, t, 1]
                ke = kc + kd
                for i in range(gs):
                    m = b0 + i - j
                    if m < 0:
                        continue
                    if m not in xw:
                        xa, xb = x_s[m, t, 0], x_s[m, t, 1]
                        xw[m] = (xa, xb, xa + xb)
                    xa, xb, xu = xw[m]
                    p = (xa * kc, xb * kd, xu * ke)
                    acc[i] = p if acc[i] is None else tuple(u + w for u, w in zip(acc[i], p))
            for i in range(gs):
                s1, s2, s3 = acc[i]
                re, im = s1 - s2, s3 - (s1 + s2)
                if prev is None:
                    zr, zi = re, im
                else:
                    zr, zi = re - prev[1], im + prev[0]
                prev = (re, im)
                z_s[b0 + i, zrows, :] = jnp.concatenate([zr, zi], axis=0).astype(BF16)
            b0 += gs

    def inv(l, t):
        rows = pl.ds(pl.multiple_of(t * BLK, BLK), BLK)
        for h, y_s in enumerate((ya_s, yb_s)):
            y_s[rows, l * 128:(l + 1) * 128] = _nn(_bf(iv_s[h]), _bf(zv[l % 2][t, h * 64:(h + 1) * 64, :]))

    def modchunk(t):
        cols = pl.ds(pl.multiple_of(jnp.minimum(t, 14) * 256, 256), 256)
        for l in range(NT):
            mp_s[l, :, cols] = _nn(_bf(cv_s[:, l * 128:(l + 1) * 128]), wm_s[l * 128:(l + 1) * 128, cols])[:8]

    for cp in kv_cps[0]:
        cp.wait()
    for u in range(UB):
        make_kv(0, u)
    ssm_cps[0].wait()

    def kv_next(l, i):
        last = i == NI - 1
        if l + 1 < NT:
            @pl.when(last)
            def _():
                for cp in kv_cps[l + 1]:
                    cp.wait()
        lt = jnp.where(last, min(l + 1, NT - 1), l)
        bt = jnp.where(last, 0, (i + 1) * UB)
        return lt, bt

    def body(i, _, l):
        if l + 1 < NT:
            lt, bt = kv_next(l + 1, i)
        for u in range(UB):
            if l + 1 < NT:
                fwd_k(l + 1, i * UB + u)
                fwd_x(l + 1, i * UB + u)
            else:
                modchunk(i * UB + u)
        if l >= 1:
            for u in range(UB):
                inv(l - 1, i * UB + u)
        if l >= 0:
            for u in range(UB):
                wconv(l, i * UB + u)
        if l + 1 < NT:
            for u in range(UB):
                make_kv(lt, bt + u)
        return 0

    for l in range(-1, NT):
        if l >= 0:
            if l + 1 < NT:
                ssm_cps[l + 1].wait()
            else:
                wm_cp.wait()
        with _scope(f"main{l}"):
            lax.fori_loop(0, NI, lambda i, c, l=l: body(i, c, l), 0)
        if l + 1 < NT:
            add_skip(l + 1)

    md = mp_s[0, 0:1, :]
    for l in range(1, NT):
        md = md + mp_s[l, 0:1, :]
    md = md.astype(BF16).astype(F32)
    sa, ca, ga, sb, cb, gb = (md[:, i * D:(i + 1) * D] for i in range(6))
    cb1 = 1.0 + cb
    wr = jnp.concatenate([wr_s[l:l + 1, :] for l in range(NT)], axis=1).astype(F32)
    u = cb1 * wr
    u_hi = u.astype(BF16)
    u_lo = (u - u_hi.astype(F32)).astype(BF16)
    rid16 = lax.broadcasted_iota(jnp.int32, (16, D), 0)
    cv_s[...] = pltpu.bitcast(
        jnp.where(rid16 == 0, u_hi.astype(F32), jnp.where(rid16 == 1, u_lo.astype(F32), 0.0)).astype(BF16), U32)
    r_off = jnp.sum(sb * wr, axis=-1, keepdims=True)
    cf_s[0] = jnp.broadcast_to((1.0 + ca) * ga, (8, D))
    cf_s[1] = jnp.broadcast_to(sa * ga, (8, D))
    cf_s[2] = jnp.broadcast_to(cb1 * gb, (8, D))
    cf_s[3] = jnp.broadcast_to(sb * gb, (8, D))

    def coef(i):
        return jnp.tile(cf_s[i], (SL // 8, 1))

    class Win:
        def __init__(self, g0, n):
            self.g0 = g0
            rows = pl.ds(g0 * RG if isinstance(g0, int) else pl.multiple_of(g0 * RG, RG), n * RG)
            self.q, self.ya, self.yb, self.xx, self.o = (r.at[rows] for r in (q_s, ya_s, yb_s, xx_s, o_s))
            self.st = st_s.at[:, rows]
            self.pt = pt_s.at[:, rows]
            self.n2 = n2_s.at[:, rows]

    def fold(x):
        acc = x[:, 0:128]
        for l in range(1, NT):
            acc = acc + x[:, l * 128:(l + 1) * 128]
        return acc

    def sums(w, x, rows, slot):
        w.pt[slot, rows, :] = fold(x)
        w.pt[slot + 1, rows, :] = fold(x * x)

    def stage_r(w, k, slot):
        rows = pl.ds(k * RG, RG)
        for j in (slot, slot + 1):
            w.st[j, rows, :] = jnp.broadcast_to(jnp.sum(w.pt[j, rows, :], axis=-1, keepdims=True), (RG, 128))

    def stats(w, rows, slot):
        m = w.st[slot, rows, :] * (1.0 / D)
        var = jnp.maximum(w.st[slot + 1, rows, :] * (1.0 / D) - m * m, 0.0)
        rs = jnp.exp2(-0.5 * jnp.log2(var + EPS))
        return jnp.tile(m, (1, NT)), jnp.tile(rs, (1, NT))

    def slices(k):
        return [pl.ds(k * RG + s * SL, SL) for s in range(RG // SL)]

    def stage_inv(w, k):
        g = w.g0 + k
        per = BLK // RG
        grows = pl.ds(pl.multiple_of((g % per) * (RG // 2), 8), RG // 2)
        for h, y in enumerate((w.ya, w.yb)):
            y[k * RG:(k + 1) * RG, (NT - 1) * 128:] = _nn(
                _bf(iv_s[h, grows, :]), _bf(zv[(NT - 1) % 2][g // per, h * 64:(h + 1) * 64, :]))

    def stage_a(w, k):
        for rows in slices(k):
            sums(w, w.q[rows, :].astype(F32), rows, 0)

    def stage_b(w, k):
        for rows in slices(k):
            m, rs = stats(w, rows, 0)
            x = w.q[rows, :].astype(F32)
            x1 = x + (w.ya[rows, :] + w.yb[rows, :]) * ((x - m) * rs * coef(0) + coef(1))
            w.xx[rows, :] = x1
            sums(w, x1, rows, 2)

    def stage_c(w, k):
        for rows in slices(k):
            m, rs = stats(w, rows, 2)
            x1 = w.xx[rows, :]
            n2 = (x1 - m) * rs
            for l in range(NT):
                w.n2[l, rows, :] = n2[:, l * 128:(l + 1) * 128].astype(BF16)
            w.o[rows, :] = (x1 + n2 * coef(2) + coef(3)).astype(BF16)

    def stage_d(g):
        rows = pl.ds(pl.multiple_of(g * (RG // 2), RG // 2), RG // 2)
        for l in range(NT):
            r_s[l, pl.ds(pl.multiple_of(g * 8, 8), 8), :] = _nt(
                _bf(cv_s[:, l * 128:(l + 1) * 128]), _bf(n2_v[l, rows, :]))[:8]

    def p2_step(g):
        static = isinstance(g, int)
        lo = max(g, 0) if static else g
        hi = min(g + 5, NG) if static else None
        w = Win(lo, hi - lo) if (static and hi > lo) else (None if static else Win(g, 5))

        def ok(d):
            return (not static) or 0 <= g + d < NG
        off = lo - g if static else 0
        if ok(-1):
            stage_d(g - 1)
        if ok(4):
            stage_inv(w, 4 - off)
        if ok(3):
            stage_r(w, 3 - off, 0)
        if ok(1):
            stage_r(w, 1 - off, 2)
        if ok(4):
            stage_a(w, 4 - off)
        if ok(2):
            stage_b(w, 2 - off)
        if ok(0):
            stage_c(w, 0 - off)

    q_cp.wait()
    with _scope("p2pro"):
        for g in range(-4, 1):
            p2_step(g)

    def p2(g, _):
        p2_step(g)
        return 0

    with _scope("p2"):
        lax.fori_loop(1, NG - 4, p2, 0)
    with _scope("p2epi"):
        for g in range(NG - 4, NG + 1):
            p2_step(g)

    r = r_off
    for l in range(NT):
        r = r + r_s[l, pl.ds(0, NG, stride=8), :] + r_s[l, pl.ds(1, NG, stride=8), :]
    tok = lax.broadcasted_iota(jnp.int32, (NG, RG), 0) * RG + lax.broadcasted_iota(jnp.int32, (NG, RG), 1)
    m1 = jnp.max(r)
    i1 = jnp.min(jnp.where(r == m1, tok, S - 1))
    r2 = jnp.where(tok == i1, -jnp.inf, r)
    m2 = jnp.max(r2)
    i2 = jnp.min(jnp.where(jnp.logical_and(r2 == m2, tok != i1), tok, S - 1))

    def grp(i):
        return pl.ds(pl.multiple_of((i // 16) * 16, 16), 16)

    def pick(i):
        blk = jnp.concatenate([n2_s[l, grp(i), :] for l in range(NT)], axis=1).astype(F32)
        return jnp.sum(jnp.where(rid16 == i % 16, blk, 0.0), axis=0, keepdims=True)

    h1 = pick(i1) * cb1 + sb
    h2 = pick(i2) * cb1 + sb
    xsel = jnp.where(rid16 == 0, h1, jnp.where(rid16 == 1, h2, 0.0)).astype(BF16)

    b1, b2 = i1 // BLK, i2 // BLK
    yacc = jnp.zeros((16, D), F32)
    for i, (st, n) in enumerate(FCH):
        for cp in f_cps[i]:
            cp.wait()
        if i == len(FCH) - 2:
            for b in range(NB):
                @pl.when(jnp.logical_and(b != b1, b != b2))
                def _():
                    o_copy(b).start()
        with _scope(f"ffn{i}"):
            g = _nt(xsel, wg_s[st:st + n, :])
            up = _nt(xsel, wu_s[st:st + n, :])
            act = (g * jax.nn.sigmoid(g) * up).astype(BF16)
            yacc = yacc + _nn(act, wd_s[st:st + n, :])

    rsel = jnp.where(rid16[:, :1] == 0, m1, m2)
    upd = yacc * jax.nn.sigmoid(rsel) * gb
    for row, i in ((0, i1), (1, i2)):
        cur = o_s[grp(i), :].astype(F32)
        o_s[grp(i), :] = (cur + jnp.where(rid16 == i % 16, upd[row:row + 1], 0.0)).astype(BF16)
    o_copy(b1).start()

    @pl.when(b2 != b1)
    def _():
        o_copy(b2).start()
    for b in range(NB):
        o_copy(b).wait()


@jax.jit
def pallas_adaLN_cond__ssm_conv_h3__moe_arch_mod__prompt_kernel(
    A_q, A_k, A_v, A_shift_k, A_ssm_k, A_ssm_D, B_x, B_w_r, B_w_gate, B_w_up, B_w_down, c, w_mod,
):
    fwd, inv = _dft_mats()
    V = pltpu.VMEM
    dma = pltpu.SemaphoreType.DMA
    spec = (NB, 16, 2, 8, 128)
    scratch = [
        V((S, D), BF16), V((NT, S, 128), BF16), V((NT, S, 128), BF16), V((4, D), BF16),
        V((D // 2, S), U32), V((NT, 128), BF16), V((NT, 128), BF16),
        V((FF // 2, D), U32), V((FF // 2, D), U32), V((FF // 2, D), U32), V((1, D), BF16),
        V((D // 2, 6 * D), U32),
        V(fwd.shape, U32), V(inv.shape, U32),
        V((S + 8, 128), F32), V((NB, BLK, 128), BF16), V((NT, 4, 8, 128), F32),
        V(spec, F32), V(spec, F32), V(spec, F32), V(spec, F32),
        V((NB, 256, 128), BF16), V((NB, 256, 128), BF16),
        V((S, D), F32), V((S, D), F32), V((NT, 8, 6 * D), F32), V((4, 8, D), F32),
        V((NT, S, 128), BF16), V((S, D), BF16), V((NT, NG * 8, RG), F32),
        V((4, S, 128), F32), V((4, S, 128), F32), V((S, D), F32), V((8, D), U32), pltpu.SMEM((8,), jnp.int32),
        dma((6 + 3 * NT + 2 + 3 * len(FCH),)), dma((NB,)),
    ]
    out = pl.pallas_call(
        _kernel,
        out_shape=jax.ShapeDtypeStruct((S, D), BF16),
        in_specs=[pl.BlockSpec(memory_space=pl.ANY)] * 14,
        out_specs=pl.BlockSpec(memory_space=pl.ANY),
        scratch_shapes=scratch,
        compiler_params=pltpu.CompilerParams(vmem_limit_bytes=100 * 1024 * 1024),
    )(A_q.reshape(S, D), A_k.reshape(S, D), A_v.reshape(S, D), A_shift_k.T, A_ssm_k,
      A_ssm_D.reshape(NT, 128), B_w_r.reshape(NT, 128), B_w_gate.T, B_w_up.T, B_w_down, c, w_mod,
      jnp.asarray(fwd), jnp.asarray(inv))
    return out.reshape(1, S, D)
```

```python
import math

import jax
import jax.numpy as jnp
from jax import lax
import jax.experimental.pallas as pl
import jax.experimental.pallas.tpu as pltpu

S, D, FF = 2048, 640, 1728
BLK = 128
NB = S // BLK
NT = D // 128
EPS = 1e-5
EPS_BF16 = 1.0013580322265625e-05
F32, BF16, U32, I32 = jnp.float32, jnp.bfloat16, jnp.uint32, jnp.int32

PCH = 8
PB = NB // PCH
UB = 2
NI = NB // UB
AR = UB * BLK
GROUPS = (5, 5, 6)
NQ = 4
RG = BLK // 2
NG = S // RG
SL = 16
WD_TAIL = 256
NSEM = 2 + PCH + NT + 1 + NQ + 2

_SPEC = (NB, 16, 2, 8, 128)
_SCRATCH = dict(
    q=((S, D), BF16), k=((S, D), BF16), v=((S, D), BF16), sk=((4, D), BF16), ssm=((D // 2, S), U32),
    dd=((NT, 128), BF16), wr=((NT, 128), BF16), wg=((FF // 2, D), U32), wu=((FF // 2, D), U32),
    wd=((FF // 2, D), U32), c=((1, D), BF16), wm=((D // 2, 6 * D), U32),
    fw=((256, 128), BF16), iv=((2, 128, 128), BF16),
    kf=((NT, S + 8, 128), F32), kv=((NT * PB, BLK, 128), BF16), tap=((NT, 4, 8, 128), F32),
    x=((NT,) + _SPEC, F32), k0=(_SPEC, F32), k1=(_SPEC, F32),
    z0=((NB, 256, 128), BF16), z1=((NB, 256, 128), BF16),
    ya=((S, D), F32), yb=((S, D), F32), mp=((NT, 8, 6 * D), F32), cf=((4, 8, D), F32),
    n2=((NT, S, 128), BF16), o=((S, D), BF16), r=((NT, NG * 8, RG), F32),
    st=((4, S, 128), F32), pt=((4, S, 128), F32), xx=((S, D), F32), cv=((8, D), U32),
)


def _nn(a, b):
    return jnp.dot(a, b, preferred_element_type=F32)


def _nt(a, b):
    return lax.dot_general(a, b, (((1,), (1,)), ((), ())), preferred_element_type=F32)


def _rb(x):
    return x.astype(BF16).astype(F32)


def _packed(ref):
    view = ref.bitcast(U32)

    def load(lead, start, size, align):
        start = start // 2 if isinstance(start, int) else pl.multiple_of(start >> 1, align // 2)
        return pltpu.bitcast(view[lead + (pl.ds(start, size // 2), slice(None))], BF16)
    return load


def _dft(freq_axis, shape, first):
    r = lax.broadcasted_iota(I32, shape, freq_axis) + first
    s = lax.broadcasted_iota(I32, shape, 1 - freq_axis)
    m = ((r >> 4) << 3) + (r & 7)
    n = ((4 * m + 1) * s + ((r >> 3) & 1) * 128) & 511
    return jnp.cos(n.astype(F32) * (math.pi / 256.0))


class _Refs:
    def __init__(self, refs):
        self.refs = dict(zip(_SCRATCH, refs))

    def __getattr__(self, name):
        return self.refs[name]


def _body(q_h, k_h, v_h, sk_h, ssm_h, dd_h, wr_h, wg_h, wu_h, wd_h, c_h, wm_h, o_h, R, zero_s, sem_o, sem_i):
    ks, zs = (R.k0, R.k1), (R.z0, R.z1)
    z_ld = (_packed(R.z0), _packed(R.z1))
    kv_ld, n2_ld, fw_ld, iv_ld = (_packed(r) for r in (R.kv, R.n2, R.fw, R.iv))
    ssm_s, wg_s, wu_s, wd_s, wm_s = (r.bitcast(BF16) for r in (R.ssm, R.wg, R.wu, R.wd, R.wm))

    def cv_tile(l):
        return pltpu.bitcast(R.cv[:, l * 128:(l + 1) * 128], BF16)

    order = []

    def group(*pairs):
        sem = sem_i.at[len(order)]
        cps = [pltpu.make_async_copy(a, b, sem) for a, b in pairs]
        order.append(cps)
        return cps

    def wait(cps):
        for cp in cps:
            cp.wait()

    def wait_at(i, table):
        for it, cps in table.items():
            @pl.when(i == it)
            def _():
                wait(cps)

    def ssm_group(l):
        rows = pl.ds(l * 128, 128)
        return group((ssm_h.at[rows], ssm_s.at[rows]))

    sk_cp = group((sk_h, R.sk))
    ssm_cps = [ssm_group(0)]
    kv_cps = []
    for c in range(PCH):
        rows = pl.ds(c * (S // PCH), S // PCH)
        kv_cps.append(group((k_h.at[rows], R.k.at[rows]), (v_h.at[rows], R.v.at[rows])))
    small = group((dd_h, R.dd), (wr_h, R.wr), (c_h, R.c))
    ssm_cps += [ssm_group(l) for l in range(1, NT)]
    wm_cp = group((wm_h, wm_s))
    q_cps = []
    for c in range(NQ):
        rows = pl.ds(c * (S // NQ), S // NQ)
        q_cps.append(group((q_h.at[rows], R.q.at[rows])))
    head, tail = pl.ds(0, FF - WD_TAIL), pl.ds(FF - WD_TAIL, WD_TAIL)
    f_head = group((wg_h, wg_s), (wu_h, wu_s), (wd_h.at[head], wd_s.at[head]))
    f_tail = group((wd_h.at[tail], wd_s.at[tail]))
    for cps in order:
        for cp in cps:
            cp.start()

    def o_copy(b):
        rows = pl.ds(pl.multiple_of(b * BLK, BLK), BLK)
        return pltpu.make_async_copy(R.o.at[rows], o_h.at[rows], sem_o)

    R.fw[...] = _dft(0, (256, 128), 0).astype(BF16)
    for h in range(2):
        R.iv[h] = (_dft(1, (128, 128), h * 128) * (1.0 / 128.0)).astype(BF16)
    for l in range(NT):
        R.kf[l, pl.ds(0, 8), :] = jnp.zeros((8, 128), F32)
    for g in range(len(GROUPS)):
        zero_s[g] = 0
    wait(sk_cp)
    skf = R.sk[...].astype(F32)
    for l in range(NT):
        for j in range(4):
            R.tap[l, j] = jnp.broadcast_to(skf[j:j + 1, l * 128:(l + 1) * 128], (8, 128))

    def make_kv(l, t, slot):
        r0 = pl.multiple_of(t * BLK, BLK)
        cols = slice(l * 128, (l + 1) * 128)
        kb = R.k[pl.ds(r0, BLK), cols].astype(F32)
        R.kf[l, pl.ds(r0 + 8, BLK), :] = kb
        w = [jnp.tile(R.tap[l, j], (BLK // 8, 1)) for j in range(4)]
        acc = kb * w[0]
        for j in range(1, 4):
            acc = acc + R.kf[l, pl.ds(r0 + 8 - j, BLK), :] * w[j]
        R.kv[slot] = (acc * R.v[pl.ds(r0, BLK), cols].astype(F32)).astype(BF16)

    def fwd_x(l, t, slot):
        R.x[l, t] = _nn(fw_ld((), 0, 256, 0), kv_ld((slot,), 0, BLK, 0)).reshape(_SPEC[1:])

    def fwd_k(l, t):
        taps = pl.ds(pl.multiple_of(t * BLK, BLK), BLK)
        ks[l % 2][t] = _nt(fw_ld((), 0, 256, 0), ssm_s[l * 128:(l + 1) * 128, taps]).reshape(_SPEC[1:])

    def add_skip(l):
        kk = ks[l % 2]
        kk[0, :, 0] = kk[0, :, 0] + R.dd[l:l + 1, :].astype(F32)

    def wconv(l, t0):
        kk, z = ks[l % 2], zs[l % 2]
        zrows = pl.ds(pl.multiple_of(t0 * 16, 16), 16)
        prev = None
        b0 = 0
        for g, gs in enumerate(GROUPS):
            t = t0 + zero_s[g]
            acc = [None] * gs
            xw = {}
            for j in range(b0 + gs):
                kc, kd = kk[j, t, 0], kk[j, t, 1]
                ke = kc + kd
                for i in range(gs):
                    m = b0 + i - j
                    if m < 0:
                        continue
                    if m not in xw:
                        xa, xb = R.x[l, m, t, 0], R.x[l, m, t, 1]
                        xw[m] = (xa, xb, xa + xb)
                    xa, xb, xu = xw[m]
                    p = (xa * kc, xb * kd, xu * ke)
                    acc[i] = p if acc[i] is None else tuple(u + w for u, w in zip(acc[i], p))
            for i in range(gs):
                s1, s2, s3 = acc[i]
                re, im = s1 - s2, s3 - (s1 + s2)
                if prev is None:
                    zr, zi = re, im
                else:
                    zr, zi = re - prev[1], im + prev[0]
                prev = (re, im)
                z[b0 + i, zrows, :] = jnp.concatenate([zr, zi], axis=0).astype(BF16)
            b0 += gs

    def inv(l, t, ya, yb, rows, g0, n):
        for h, y in enumerate((ya, yb)):
            y[rows, l * 128:(l + 1) * 128] = _nn(iv_ld((h,), g0, n, n), z_ld[l % 2]((t,), h * 128, 128, 0))

    def modchunk(t):
        cols = pl.ds(pl.multiple_of(jnp.minimum(t, 14) * 256, 256), 256)
        for l in range(NT):
            R.mp[l, :, cols] = _nn(cv_tile(l), wm_s[l * 128:(l + 1) * 128, cols])[:8]

    class Win:
        def __init__(self, r0, n):
            rows = pl.ds(r0 if isinstance(r0, int) else pl.multiple_of(r0, RG), n)
            self.q, self.ya, self.yb, self.xx, self.o = (r.at[rows] for r in (R.q, R.ya, R.yb, R.xx, R.o))
            self.st, self.pt, self.n2 = (r.at[:, rows] for r in (R.st, R.pt, R.n2))

    def fold(x):
        acc = x[:, 0:128]
        for l in range(1, NT):
            acc = acc + x[:, l * 128:(l + 1) * 128]
        return acc

    def sums(w, x, rows, slot):
        w.pt[slot, rows, :] = fold(x)
        w.pt[slot + 1, rows, :] = fold(x * x)

    def stage_r(w, r0, n, slot):
        rows = pl.ds(r0, n)
        for j in (slot, slot + 1):
            w.st[j, rows, :] = jnp.broadcast_to(jnp.sum(w.pt[j, rows, :], axis=-1, keepdims=True), (n, 128))

    def stage_a(w, n):
        for s in range(n // SL):
            rows = pl.ds(s * SL, SL)
            sums(w, w.q[rows, :].astype(F32), rows, 0)

    wait(ssm_cps[0])

    def p0(i, _):
        wait_at(i, dict(enumerate(kv_cps)))
        for u in range(PB):
            fwd_k(0, i * PB + u)
        for u in range(PB):
            for l in range(NT):
                make_kv(l, i * PB + u, u * NT + l)
                fwd_x(l, i * PB + u, u * NT + l)
        return 0

    lax.fori_loop(0, PCH, p0, 0)
    wait(small)
    add_skip(0)
    cvec = R.c[...].astype(F32)
    R.cv[...] = pltpu.bitcast(jnp.broadcast_to((cvec * _rb(jax.nn.sigmoid(cvec))).astype(BF16), (16, D)), U32)

    def p1(i, l):
        last = l + 1 == NT
        if last:
            wait_at(i, {(c * (S // NQ)) // AR: q_cps[c] for c in range(NQ)})
        for u in range(UB):
            if last:
                modchunk(i * UB + u)
            else:
                fwd_k(l + 1, i * UB + u)
        if l >= 1:
            for u in range(UB):
                t = i * UB + u
                inv(l - 1, t, R.ya, R.yb, pl.ds(pl.multiple_of(t * BLK, BLK), BLK), 0, BLK)
        if last:
            stage_r(Win(jnp.maximum(i - 1, 0) * AR, AR), 0, AR, 0)
        for u in range(UB):
            wconv(l, i * UB + u)
        if last:
            stage_a(Win(i * AR, AR), AR)
        return 0

    for l in range(NT):
        if l + 1 < NT:
            wait(ssm_cps[l + 1])
        else:
            wait(wm_cp)
            R.pt[0:2, 0:AR, :] = jnp.zeros((2, AR, 128), F32)
        lax.fori_loop(0, NI, lambda i, _, l=l: p1(i, l), 0)
        if l + 1 < NT:
            add_skip(l + 1)
    stage_r(Win(S - AR, AR), 0, AR, 0)

    md = R.mp[0, 0:1, :]
    for l in range(1, NT):
        md = md + R.mp[l, 0:1, :]
    md = _rb(md)
    sa, ca, ga, sb, cb, gb = (md[:, i * D:(i + 1) * D] for i in range(6))
    ca1, cb1 = _rb(1.0 + ca), _rb(1.0 + cb)
    wr = jnp.concatenate([R.wr[l:l + 1, :] for l in range(NT)], axis=1).astype(F32)
    u_all = cb1 * wr
    u_hi = _rb(u_all)
    rid16 = lax.broadcasted_iota(I32, (16, D), 0)
    R.cv[...] = pltpu.bitcast(
        jnp.where(rid16 == 0, u_hi, jnp.where(rid16 == 1, u_all - u_hi, 0.0)).astype(BF16), U32)
    r_off = jnp.sum(sb * wr, axis=-1, keepdims=True)
    for i, vec in enumerate((ca1 * ga, sa * ga, cb1 * gb, sb * gb)):
        R.cf[i] = jnp.broadcast_to(vec, (8, D))

    def coef(i):
        return jnp.tile(R.cf[i], (SL // 8, 1))

    def wide(a):
        return jnp.tile(a, (1, NT))

    def stats(w, rows, slot):
        m = w.st[slot, rows, :] * (1.0 / D)
        var = jnp.maximum(w.st[slot + 1, rows, :] * (1.0 / D) - m * m, 0.0)
        return m, jnp.exp2(jnp.log(var + EPS) * (-0.5 / math.log(2.0)))

    def slice_b(w, rows, m, rs):
        x = w.q[rows, :].astype(F32)
        x1 = x + (w.ya[rows, :] + w.yb[rows, :]) * ((x - wide(m)) * wide(rs) * coef(0) + coef(1))
        w.xx[rows, :] = x1
        sums(w, x1, rows, 2)

    def slice_c(w, rows, m, rs):
        x1 = w.xx[rows, :]
        n2 = (x1 - wide(m)) * wide(rs)
        for l in range(NT):
            w.n2[l, rows, :] = n2[:, l * 128:(l + 1) * 128].astype(BF16)
        w.o[rows, :] = (x1 + n2 * coef(2) + coef(3)).astype(BF16)

    def stage_bc(w, kb, kc):
        tasks = []
        for fn, k, slot in ((slice_b, kb, 0), (slice_c, kc, 2)):
            if k is not None:
                tasks += [(fn, pl.ds(k * RG + s * SL, SL), slot) for s in range(RG // SL)]
        nxt = stats(w, *tasks[0][1:])
        for i, (fn, rows, _) in enumerate(tasks):
            cur = nxt
            if i + 1 < len(tasks):
                nxt = stats(w, *tasks[i + 1][1:])
            fn(w, rows, *cur)

    def stage_d(g):
        for l in range(NT):
            R.r[l, pl.ds(pl.multiple_of(g * 8, 8), 8), :] = _nt(cv_tile(l), n2_ld((l,), g * RG, RG, RG))[:8]

    def p2_step(g):
        static = isinstance(g, int)
        lo = max(g, 0) if static else g
        n = (min(g + 4, NG) - lo) if static else 4
        w = Win(lo * RG, n * RG) if n > 0 else None
        off = lo - g if static else 0

        def ok(d):
            return (not static) or 0 <= g + d < NG
        if ok(-1):
            stage_d(g - 1)
        if ok(3):
            inv(NT - 1, (g + 3) >> 1, w.ya, w.yb, pl.ds((3 - off) * RG, RG), ((g + 3) & 1) * RG, RG)
        if ok(1):
            stage_r(w, (1 - off) * RG, RG, 2)
        if ok(2) or ok(0):
            stage_bc(w, 2 - off if ok(2) else None, 0 - off if ok(0) else None)
        return 0

    for g in range(-3, 1):
        p2_step(g)
    lax.fori_loop(1, NG - 3, lambda g, _: p2_step(g), 0)
    for g in range(NG - 3, NG + 1):
        p2_step(g)

    r = jnp.broadcast_to(r_off, (NG, RG))
    for l in range(NT):
        r = r + R.r[l, pl.ds(0, NG, stride=8), :] + R.r[l, pl.ds(1, NG, stride=8), :]
    tok = lax.broadcasted_iota(I32, (NG, RG), 0) * RG + lax.broadcasted_iota(I32, (NG, RG), 1)
    bits = lax.bitcast_convert_type(r, I32)
    key = lax.bitcast_convert_type((bits & ~(S - 1)) | jnp.where(bits < 0, tok, S - 1 - tok), F32)

    def amax(x):
        return jnp.max(jnp.max(x, axis=0, keepdims=True), axis=1, keepdims=True)

    def index_of(kv):
        kb = lax.bitcast_convert_type(kv, I32)
        low = kb & (S - 1)
        return jnp.where(kb < 0, low, S - 1 - low)[0, 0]

    m1 = amax(key)
    m2 = amax(jnp.where(key == m1, -jnp.inf, key))
    i1, i2 = index_of(m1), index_of(m2)
    b1, b2 = i1 >> 7, i2 >> 7

    wait(f_head)
    for b in range(NB):
        @pl.when(jnp.logical_and(b != b1, b != b2))
        def _():
            o_copy(b).start()

    def grp(i):
        return pl.ds(pl.multiple_of((i >> 4) << 4, 16), 16)

    def two_rows(f):
        return jnp.where(rid16 == 0, f(i1), jnp.where(rid16 == 1, f(i2), 0.0))

    def q_row(i):
        return jnp.sum(jnp.where(rid16 == (i & 15), R.q[grp(i), :].astype(F32), 0.0), axis=0, keepdims=True)

    def ln_rows(x):
        m = jnp.mean(x, axis=-1, keepdims=True)
        var = jnp.mean(jnp.square(x - m), axis=-1, keepdims=True)
        return _rb(_rb(x - _rb(m)) / _rb(jnp.sqrt(_rb(_rb(var) + EPS_BF16))))

    xq = two_rows(q_row)
    yr = _rb(two_rows(lambda i: R.ya[pl.ds(i, 1), :] + R.yb[pl.ds(i, 1), :]))
    hq = _rb(_rb(ln_rows(xq) * ca1) + sa)
    x1r = _rb(xq + _rb(ga * _rb(hq * yr)))
    hr = _rb(_rb(ln_rows(x1r) * cb1) + sb)
    xsel = hr.astype(BF16)
    gate = _rb(_nt(xsel, wg_s[...]))
    up = _rb(_nt(xsel, wu_s[...]))
    act = (_rb(gate * _rb(jax.nn.sigmoid(gate))) * up).astype(BF16)
    wait(f_tail)
    yf = _rb(_nn(act, wd_s[...]))
    rsel = _rb(jax.nn.sigmoid(_rb(jnp.where(rid16[:, :1] == 0, m1, m2))))
    fin = x1r + _rb(gb * _rb(hr + _rb(yf * rsel)))
    for row, i in ((0, i1), (1, i2)):
        cur = R.o[grp(i), :].astype(F32)
        R.o[grp(i), :] = jnp.where(rid16 == (i & 15), fin[row:row + 1], cur).astype(BF16)
    o_copy(b1).start()

    @pl.when(b2 != b1)
    def _():
        o_copy(b2).start()


def _kernel(*refs):
    ins, o_h, scr = refs[:12], refs[12], refs[13:]
    R = _Refs(scr)
    zero_s, sem_o = scr[-2], scr[-1]
    pl.run_scoped(lambda sem_i: _body(*ins, o_h, R, zero_s, sem_o, sem_i), pltpu.SemaphoreType.DMA((NSEM,)))
    pltpu.make_async_copy(R.o, o_h, sem_o).wait()


@jax.jit
def pallas_adaLN_cond__ssm_conv_h3__moe_arch_mod__prompt_kernel(
    A_q: jax.Array,
    A_k: jax.Array,
    A_v: jax.Array,
    A_shift_k: jax.Array,
    A_ssm_k: jax.Array,
    A_ssm_D: jax.Array,
    B_x: jax.Array,
    B_w_r: jax.Array,
    B_w_gate: jax.Array,
    B_w_up: jax.Array,
    B_w_down: jax.Array,
    c: jax.Array,
    w_mod: jax.Array,
):
    scratch = [pltpu.VMEM(shape, dt) for shape, dt in _SCRATCH.values()]
    scratch += [pltpu.SMEM((len(GROUPS),), I32), pltpu.SemaphoreType.DMA(())]
    out = pl.pallas_call(
        _kernel,
        out_shape=jax.ShapeDtypeStruct((S, D), BF16),
        in_specs=[pl.BlockSpec(memory_space=pl.ANY)] * 12,
        out_specs=pl.BlockSpec(memory_space=pl.ANY),
        scratch_shapes=scratch,
        compiler_params=pltpu.CompilerParams(vmem_limit_bytes=100 * 1024 * 1024),
    )(A_q.reshape(S, D), A_k.reshape(S, D), A_v.reshape(S, D), A_shift_k.T, A_ssm_k,
      A_ssm_D.reshape(NT, 128), B_w_r.reshape(NT, 128), B_w_gate.T, B_w_up.T, B_w_down, c, w_mod)
    return out.reshape(1, S, D)
```

```python
import math

import jax
import jax.numpy as jnp
from jax import lax
import jax.experimental.pallas as pl
import jax.experimental.pallas.tpu as pltpu

S, D, FF = 2048, 640, 1728
BLK = 128
NB = S // BLK
NT = D // 128
EPS = 1e-5
EPS_BF16 = 1.0013580322265625e-05
F32, BF16, U32, I32 = jnp.float32, jnp.bfloat16, jnp.uint32, jnp.int32

PCH = 8
PB = NB // PCH
UB = 2
NI = NB // UB
AR = UB * BLK
GROUPS = (5, 5, 6)
NQ = 4
RG = BLK // 2
NG = S // RG
SL = 16
WD_TAIL = 256
NSEM = 2 + PCH + NT + 1 + NQ + 2

_SPEC = (NB, 16, 2, 8, 128)
_SCRATCH = dict(
    q=((S, D), BF16), k=((S, D), BF16), v=((S, D), BF16), sk=((4, D), BF16), ssm=((D // 2, S), U32),
    dd=((NT, 128), BF16), wr=((NT, 128), BF16), wg=((FF // 2, D), U32), wu=((FF // 2, D), U32),
    wd=((FF // 2, D), U32), c=((1, D), BF16), wm=((D // 2, 6 * D), U32),
    fw=((256, 128), BF16), iv=((2, 128, 128), BF16),
    kf=((NT, S + 8, 128), F32), kv=((NT * PB, BLK, 128), BF16), tap=((NT, 4, 8, 128), F32),
    x=((NT,) + _SPEC, F32), k0=(_SPEC, F32), k1=(_SPEC, F32),
    z0=((NB, 256, 128), BF16), z1=((NB, 256, 128), BF16),
    ya=((S, D), F32), yb=((S, D), F32), mp=((NT, 8, 6 * D), F32), cf=((4, 8, D), F32),
    n2=((NT, S, 128), BF16), o=((S, D), BF16), r=((NT, NG * 8, RG), F32),
    st=((4, S, 128), F32), pt=((4, S, 128), F32), xx=((S, D), F32), cv=((8, D), U32),
)


def _nn(a, b):
    return jnp.dot(a, b, preferred_element_type=F32)


def _nt(a, b):
    return lax.dot_general(a, b, (((1,), (1,)), ((), ())), preferred_element_type=F32)


def _rb(x):
    return x.astype(BF16).astype(F32)


def _sigmoid_bf16(x):
    return _rb(1.0 / _rb(1.0 + _rb(jnp.exp(-x))))


def _packed(ref):
    view = ref.bitcast(U32)

    def load(lead, start, size, align):
        start = start // 2 if isinstance(start, int) else pl.multiple_of(start >> 1, align // 2)
        return pltpu.bitcast(view[lead + (pl.ds(start, size // 2), slice(None))], BF16)
    return load


def _dft(freq_axis, shape, first):
    r = lax.broadcasted_iota(I32, shape, freq_axis) + first
    s = lax.broadcasted_iota(I32, shape, 1 - freq_axis)
    m = ((r >> 4) << 3) + (r & 7)
    n = ((4 * m + 1) * s + ((r >> 3) & 1) * 128) & 511
    return jnp.cos(n.astype(F32) * (math.pi / 256.0))


class _Refs:
    def __init__(self, refs):
        self.refs = dict(zip(_SCRATCH, refs))

    def __getattr__(self, name):
        return self.refs[name]


def _body(q_h, k_h, v_h, sk_h, ssm_h, dd_h, wr_h, wg_h, wu_h, wd_h, c_h, wm_h, o_h, R, zero_s, sem_o, sem_i):
    ks, zs = (R.k0, R.k1), (R.z0, R.z1)
    z_ld = (_packed(R.z0), _packed(R.z1))
    kv_ld, n2_ld, fw_ld, iv_ld = (_packed(r) for r in (R.kv, R.n2, R.fw, R.iv))
    ssm_s, wg_s, wu_s, wd_s, wm_s = (r.bitcast(BF16) for r in (R.ssm, R.wg, R.wu, R.wd, R.wm))

    def cv_tile(l):
        return pltpu.bitcast(R.cv[:, l * 128:(l + 1) * 128], BF16)

    order = []

    def group(*pairs):
        sem = sem_i.at[len(order)]
        cps = [pltpu.make_async_copy(a, b, sem) for a, b in pairs]
        order.append(cps)
        return cps

    def wait(cps):
        for cp in cps:
            cp.wait()

    def wait_at(i, table):
        for it, cps in table.items():
            @pl.when(i == it)
            def _():
                wait(cps)

    def ssm_group(l):
        rows = pl.ds(l * 128, 128)
        return group((ssm_h.at[rows], ssm_s.at[rows]))

    sk_cp = group((sk_h, R.sk))
    ssm_cps = [ssm_group(0)]
    kv_cps = []
    for c in range(PCH):
        rows = pl.ds(c * (S // PCH), S // PCH)
        kv_cps.append(group((k_h.at[rows], R.k.at[rows]), (v_h.at[rows], R.v.at[rows])))
    small = group((dd_h, R.dd), (wr_h, R.wr), (c_h, R.c))
    ssm_cps += [ssm_group(l) for l in range(1, NT)]
    wm_cp = group((wm_h, wm_s))
    q_cps = []
    for c in range(NQ):
        rows = pl.ds(c * (S // NQ), S // NQ)
        q_cps.append(group((q_h.at[rows], R.q.at[rows])))
    head, tail = pl.ds(0, FF - WD_TAIL), pl.ds(FF - WD_TAIL, WD_TAIL)
    f_head = group((wg_h, wg_s), (wu_h, wu_s), (wd_h.at[head], wd_s.at[head]))
    f_tail = group((wd_h.at[tail], wd_s.at[tail]))
    for cps in order:
        for cp in cps:
            cp.start()

    def o_copy(b):
        rows = pl.ds(pl.multiple_of(b * BLK, BLK), BLK)
        return pltpu.make_async_copy(R.o.at[rows], o_h.at[rows], sem_o)

    R.fw[...] = _dft(0, (256, 128), 0).astype(BF16)
    for h in range(2):
        R.iv[h] = (_dft(1, (128, 128), h * 128) * (1.0 / 128.0)).astype(BF16)
    for l in range(NT):
        R.kf[l, pl.ds(0, 8), :] = jnp.zeros((8, 128), F32)
    for g in range(len(GROUPS)):
        zero_s[g] = 0
    wait(sk_cp)
    skf = R.sk[...].astype(F32)
    for l in range(NT):
        for j in range(4):
            R.tap[l, j] = jnp.broadcast_to(skf[j:j + 1, l * 128:(l + 1) * 128], (8, 128))

    def make_kv(l, t, slot):
        r0 = pl.multiple_of(t * BLK, BLK)
        cols = slice(l * 128, (l + 1) * 128)
        kb = R.k[pl.ds(r0, BLK), cols].astype(F32)
        R.kf[l, pl.ds(r0 + 8, BLK), :] = kb
        w = [jnp.tile(R.tap[l, j], (BLK // 8, 1)) for j in range(4)]
        acc = kb * w[0]
        for j in range(1, 4):
            acc = acc + R.kf[l, pl.ds(r0 + 8 - j, BLK), :] * w[j]
        R.kv[slot] = (acc * R.v[pl.ds(r0, BLK), cols].astype(F32)).astype(BF16)

    def fwd_x(l, t, slot):
        R.x[l, t] = _nn(fw_ld((), 0, 256, 0), kv_ld((slot,), 0, BLK, 0)).reshape(_SPEC[1:])

    def fwd_k(l, t):
        taps = pl.ds(pl.multiple_of(t * BLK, BLK), BLK)
        ks[l % 2][t] = _nt(fw_ld((), 0, 256, 0), ssm_s[l * 128:(l + 1) * 128, taps]).reshape(_SPEC[1:])

    def add_skip(l):
        kk = ks[l % 2]
        kk[0, :, 0] = kk[0, :, 0] + R.dd[l:l + 1, :].astype(F32)

    def wconv(l, t0):
        kk, z = ks[l % 2], zs[l % 2]
        zrows = pl.ds(pl.multiple_of(t0 * 16, 16), 16)
        prev = None
        b0 = 0
        for g, gs in enumerate(GROUPS):
            t = t0 + zero_s[g]
            acc = [None] * gs
            xw = {}
            for j in range(b0 + gs):
                kc, kd = kk[j, t, 0], kk[j, t, 1]
                ke = kc + kd
                for i in range(gs):
                    m = b0 + i - j
                    if m < 0:
                        continue
                    if m not in xw:
                        xa, xb = R.x[l, m, t, 0], R.x[l, m, t, 1]
                        xw[m] = (xa, xb, xa + xb)
                    xa, xb, xu = xw[m]
                    p = (xa * kc, xb * kd, xu * ke)
                    acc[i] = p if acc[i] is None else tuple(u + w for u, w in zip(acc[i], p))
            for i in range(gs):
                s1, s2, s3 = acc[i]
                re, im = s1 - s2, s3 - (s1 + s2)
                if prev is None:
                    zr, zi = re, im
                else:
                    zr, zi = re - prev[1], im + prev[0]
                prev = (re, im)
                z[b0 + i, zrows, :] = jnp.concatenate([zr, zi], axis=0).astype(BF16)
            b0 += gs

    def inv(l, t, ya, yb, rows, g0, n):
        for h, y in enumerate((ya, yb)):
            y[rows, l * 128:(l + 1) * 128] = _nn(iv_ld((h,), g0, n, n), z_ld[l % 2]((t,), h * 128, 128, 0))

    def modchunk(t):
        cols = pl.ds(pl.multiple_of(jnp.minimum(t, 14) * 256, 256), 256)
        for l in range(NT):
            R.mp[l, :, cols] = _nn(cv_tile(l), wm_s[l * 128:(l + 1) * 128, cols])[:8]

    class Win:
        def __init__(self, r0, n):
            rows = pl.ds(r0 if isinstance(r0, int) else pl.multiple_of(r0, RG), n)
            self.q, self.ya, self.yb, self.xx, self.o = (r.at[rows] for r in (R.q, R.ya, R.yb, R.xx, R.o))
            self.st, self.pt, self.n2 = (r.at[:, rows] for r in (R.st, R.pt, R.n2))

    def fold(x):
        acc = x[:, 0:128]
        for l in range(1, NT):
            acc = acc + x[:, l * 128:(l + 1) * 128]
        return acc

    def sums(w, x, rows, slot):
        w.pt[slot, rows, :] = fold(x)
        w.pt[slot + 1, rows, :] = fold(x * x)

    def stage_r(w, r0, n, slot):
        rows = pl.ds(r0, n)
        for j in (slot, slot + 1):
            w.st[j, rows, :] = jnp.broadcast_to(jnp.sum(w.pt[j, rows, :], axis=-1, keepdims=True), (n, 128))

    def stage_a(w, n):
        for s in range(n // SL):
            rows = pl.ds(s * SL, SL)
            sums(w, w.q[rows, :].astype(F32), rows, 0)

    wait(ssm_cps[0])

    def p0(i, _):
        wait_at(i, dict(enumerate(kv_cps)))
        for u in range(PB):
            fwd_k(0, i * PB + u)
        for u in range(PB):
            for l in range(NT):
                make_kv(l, i * PB + u, u * NT + l)
                fwd_x(l, i * PB + u, u * NT + l)
        return 0

    lax.fori_loop(0, PCH, p0, 0)
    wait(small)
    add_skip(0)
    cvec = R.c[...].astype(F32)
    R.cv[...] = pltpu.bitcast(jnp.broadcast_to((cvec * _sigmoid_bf16(cvec)).astype(BF16), (16, D)), U32)

    def p1(i, l):
        last = l + 1 == NT
        if last:
            wait_at(i, {(c * (S // NQ)) // AR: q_cps[c] for c in range(NQ)})
        for u in range(UB):
            if last:
                modchunk(i * UB + u)
            else:
                fwd_k(l + 1, i * UB + u)
        if l >= 1:
            for u in range(UB):
                t = i * UB + u
                inv(l - 1, t, R.ya, R.yb, pl.ds(pl.multiple_of(t * BLK, BLK), BLK), 0, BLK)
        if last:
            stage_r(Win(jnp.maximum(i - 1, 0) * AR, AR), 0, AR, 0)
        for u in range(UB):
            wconv(l, i * UB + u)
        if last:
            stage_a(Win(i * AR, AR), AR)
        return 0

    for l in range(NT):
        if l + 1 < NT:
            wait(ssm_cps[l + 1])
        else:
            wait(wm_cp)
            R.pt[0:2, 0:AR, :] = jnp.zeros((2, AR, 128), F32)
        lax.fori_loop(0, NI, lambda i, _, l=l: p1(i, l), 0)
        if l + 1 < NT:
            add_skip(l + 1)
    stage_r(Win(S - AR, AR), 0, AR, 0)

    md = R.mp[0, 0:1, :]
    for l in range(1, NT):
        md = md + R.mp[l, 0:1, :]
    md = _rb(md)
    sa, ca, ga, sb, cb, gb = (md[:, i * D:(i + 1) * D] for i in range(6))
    ca1, cb1 = _rb(1.0 + ca), _rb(1.0 + cb)
    wr = jnp.concatenate([R.wr[l:l + 1, :] for l in range(NT)], axis=1).astype(F32)
    u_all = cb1 * wr
    u_hi = _rb(u_all)
    rid16 = lax.broadcasted_iota(I32, (16, D), 0)
    R.cv[...] = pltpu.bitcast(
        jnp.where(rid16 == 0, u_hi, jnp.where(rid16 == 1, u_all - u_hi, 0.0)).astype(BF16), U32)
    r_off = jnp.sum(sb * wr, axis=-1, keepdims=True)
    for i, vec in enumerate((ca1 * ga, sa * ga, cb1 * gb, sb * gb)):
        R.cf[i] = jnp.broadcast_to(vec, (8, D))

    def coef(i):
        return jnp.tile(R.cf[i], (SL // 8, 1))

    def wide(a):
        return jnp.tile(a, (1, NT))

    def stats(w, rows, slot):
        m = w.st[slot, rows, :] * (1.0 / D)
        var = jnp.maximum(w.st[slot + 1, rows, :] * (1.0 / D) - m * m, 0.0)
        return m, jnp.exp2(jnp.log(var + EPS) * (-0.5 / math.log(2.0)))

    def slice_b(w, rows, m, rs):
        x = w.q[rows, :].astype(F32)
        x1 = x + (w.ya[rows, :] + w.yb[rows, :]) * ((x - wide(m)) * wide(rs) * coef(0) + coef(1))
        w.xx[rows, :] = x1
        sums(w, x1, rows, 2)

    def slice_c(w, rows, m, rs):
        x1 = w.xx[rows, :]
        n2 = (x1 - wide(m)) * wide(rs)
        for l in range(NT):
            w.n2[l, rows, :] = n2[:, l * 128:(l + 1) * 128].astype(BF16)
        w.o[rows, :] = (x1 + n2 * coef(2) + coef(3)).astype(BF16)

    def stage_bc(w, kb, kc):
        tasks = []
        for fn, k, slot in ((slice_b, kb, 0), (slice_c, kc, 2)):
            if k is not None:
                tasks += [(fn, pl.ds(k * RG + s * SL, SL), slot) for s in range(RG // SL)]
        nxt = stats(w, *tasks[0][1:])
        for i, (fn, rows, _) in enumerate(tasks):
            cur = nxt
            if i + 1 < len(tasks):
                nxt = stats(w, *tasks[i + 1][1:])
            fn(w, rows, *cur)

    def stage_d(g):
        for l in range(NT):
            R.r[l, pl.ds(pl.multiple_of(g * 8, 8), 8), :] = _nt(cv_tile(l), n2_ld((l,), g * RG, RG, RG))[:8]

    def p2_step(g):
        static = isinstance(g, int)
        lo = max(g, 0) if static else g
        n = (min(g + 4, NG) - lo) if static else 4
        w = Win(lo * RG, n * RG) if n > 0 else None
        off = lo - g if static else 0

        def ok(d):
            return (not static) or 0 <= g + d < NG
        if ok(-1):
            stage_d(g - 1)
        if ok(3):
            inv(NT - 1, (g + 3) >> 1, w.ya, w.yb, pl.ds((3 - off) * RG, RG), ((g + 3) & 1) * RG, RG)
        if ok(1):
            stage_r(w, (1 - off) * RG, RG, 2)
        if ok(2) or ok(0):
            stage_bc(w, 2 - off if ok(2) else None, 0 - off if ok(0) else None)
        return 0

    for g in range(-3, 1):
        p2_step(g)
    lax.fori_loop(1, NG - 3, lambda g, _: p2_step(g), 0)
    for g in range(NG - 3, NG + 1):
        p2_step(g)

    r = jnp.broadcast_to(r_off, (NG, RG))
    for l in range(NT):
        r = r + R.r[l, pl.ds(0, NG, stride=8), :] + R.r[l, pl.ds(1, NG, stride=8), :]
    tok = lax.broadcasted_iota(I32, (NG, RG), 0) * RG + lax.broadcasted_iota(I32, (NG, RG), 1)
    bits = lax.bitcast_convert_type(r, I32)
    key = lax.bitcast_convert_type((bits & ~(S - 1)) | jnp.where(bits < 0, tok, S - 1 - tok), F32)

    def amax(x):
        return jnp.max(jnp.max(x, axis=0, keepdims=True), axis=1, keepdims=True)

    def index_of(kv):
        kb = lax.bitcast_convert_type(kv, I32)
        low = kb & (S - 1)
        return jnp.where(kb < 0, low, S - 1 - low)[0, 0]

    m1 = amax(key)
    m2 = amax(jnp.where(key == m1, -jnp.inf, key))
    i1, i2 = index_of(m1), index_of(m2)
    b1, b2 = i1 >> 7, i2 >> 7

    wait(f_head)
    for b in range(NB):
        @pl.when(jnp.logical_and(b != b1, b != b2))
        def _():
            o_copy(b).start()

    def grp(i):
        return pl.ds(pl.multiple_of((i >> 4) << 4, 16), 16)

    def two_rows(f):
        return jnp.where(rid16 == 0, f(i1), jnp.where(rid16 == 1, f(i2), 0.0))

    def q_row(i):
        return jnp.sum(jnp.where(rid16 == (i & 15), R.q[grp(i), :].astype(F32), 0.0), axis=0, keepdims=True)

    def ln_rows(x):
        m = jnp.mean(x, axis=-1, keepdims=True)
        var = jnp.mean(jnp.square(x - m), axis=-1, keepdims=True)
        return _rb(_rb(x - _rb(m)) / _rb(jnp.sqrt(_rb(_rb(var) + EPS_BF16))))

    xq = two_rows(q_row)
    yr = _rb(two_rows(lambda i: R.ya[pl.ds(i, 1), :] + R.yb[pl.ds(i, 1), :]))
    hq = _rb(_rb(ln_rows(xq) * ca1) + sa)
    x1r = _rb(xq + _rb(ga * _rb(hq * yr)))
    hr = _rb(_rb(ln_rows(x1r) * cb1) + sb)
    xsel = hr.astype(BF16)
    gate = _rb(_nt(xsel, wg_s[...]))
    up = _rb(_nt(xsel, wu_s[...]))
    act = (_rb(gate * _sigmoid_bf16(gate)) * up).astype(BF16)
    wait(f_tail)
    yf = _rb(_nn(act, wd_s[...]))
    rsel = _sigmoid_bf16(_rb(jnp.where(rid16[:, :1] == 0, m1, m2)))
    fin = x1r + _rb(gb * _rb(hr + _rb(yf * rsel)))
    for row, i in ((0, i1), (1, i2)):
        cur = R.o[grp(i), :].astype(F32)
        R.o[grp(i), :] = jnp.where(rid16 == (i & 15), fin[row:row + 1], cur).astype(BF16)
    o_copy(b1).start()

    @pl.when(b2 != b1)
    def _():
        o_copy(b2).start()


def _kernel(*refs):
    ins, o_h, scr = refs[:12], refs[12], refs[13:]
    R = _Refs(scr)
    zero_s, sem_o = scr[-2], scr[-1]
    pl.run_scoped(lambda sem_i: _body(*ins, o_h, R, zero_s, sem_o, sem_i), pltpu.SemaphoreType.DMA((NSEM,)))
    pltpu.make_async_copy(R.o, o_h, sem_o).wait()


@jax.jit
def pallas_adaLN_cond__ssm_conv_h3__moe_arch_mod__prompt_kernel(
    A_q: jax.Array,
    A_k: jax.Array,
    A_v: jax.Array,
    A_shift_k: jax.Array,
    A_ssm_k: jax.Array,
    A_ssm_D: jax.Array,
    B_x: jax.Array,
    B_w_r: jax.Array,
    B_w_gate: jax.Array,
    B_w_up: jax.Array,
    B_w_down: jax.Array,
    c: jax.Array,
    w_mod: jax.Array,
):
    scratch = [pltpu.VMEM(shape, dt) for shape, dt in _SCRATCH.values()]
    scratch += [pltpu.SMEM((len(GROUPS),), I32), pltpu.SemaphoreType.DMA(())]
    out = pl.pallas_call(
        _kernel,
        out_shape=jax.ShapeDtypeStruct((S, D), BF16),
        in_specs=[pl.BlockSpec(memory_space=pl.ANY)] * 12,
        out_specs=pl.BlockSpec(memory_space=pl.ANY),
        scratch_shapes=scratch,
        compiler_params=pltpu.CompilerParams(vmem_limit_bytes=100 * 1024 * 1024),
    )(A_q.reshape(S, D), A_k.reshape(S, D), A_v.reshape(S, D), A_shift_k.T, A_ssm_k,
      A_ssm_D.reshape(NT, 128), B_w_r.reshape(NT, 128), B_w_gate.T, B_w_up.T, B_w_down, c, w_mod)
    return out.reshape(1, S, D)
```

```python
import math

import jax
import jax.numpy as jnp
from jax import lax
import jax.experimental.pallas as pl
import jax.experimental.pallas.tpu as pltpu

S, D, FF = 2048, 640, 1728
BLK = 128
NB = S // BLK
NT = D // 128
EPS = 1e-5
EPS_BF16 = 1.0013580322265625e-05
F32, BF16, U32, I32 = jnp.float32, jnp.bfloat16, jnp.uint32, jnp.int32

PCH = 8
PB = NB // PCH
UB = 2
NI = NB // UB
AR = UB * BLK
GROUPS = (5, 5, 6)
NQ = 4
RG = BLK // 2
NG = S // RG
SL = 16
WD_TAIL = 256
NSEM = 2 + PCH + NT + 1 + NQ + 2

_SPEC = (NB, 16, 2, 8, 128)
_SCRATCH = dict(
    q=((S, D), BF16), k=((S, D), BF16), v=((S, D), BF16), sk=((4, D), BF16), ssm=((D // 2, S), U32),
    dd=((NT, 128), BF16), wr=((NT, 128), BF16), wg=((FF, D), BF16), wu=((FF, D), BF16),
    wd=((FF, D), BF16), c=((1, D), BF16), wm=((D // 2, 6 * D), U32),
    fw=((256, 128), BF16), iv=((2, 128, 128), BF16),
    kf=((NT, S + 8, 128), F32), kv=((NT * PB, BLK, 128), BF16), tap=((NT, 4, 8, 128), F32),
    x=((NT,) + _SPEC, F32), k0=(_SPEC, F32), k1=(_SPEC, F32),
    z0=((NB, 256, 128), BF16), z1=((NB, 256, 128), BF16),
    ya=((S, D), F32), yb=((S, D), F32), mp=((NT, 8, 6 * D), F32), cf=((4, 8, D), F32),
    n2=((NT, S, 128), BF16), o=((S, D), BF16), r=((NT, NG * 8, RG), F32),
    st=((4, S, 128), F32), pt=((4, S, 128), F32), xx=((S, D), F32), cv=((8, D), U32),
)


def _nn(a, b):
    return jnp.dot(a, b, preferred_element_type=F32)


def _nt(a, b):
    return lax.dot_general(a, b, (((1,), (1,)), ((), ())), preferred_element_type=F32)


def _rb(x):
    return x.astype(BF16).astype(F32)


def _sigmoid_bf16(x):
    return _rb(1.0 / _rb(1.0 + _rb(jnp.exp(-x))))


def _packed(ref):
    view = ref.bitcast(U32)

    def load(lead, start, size, align):
        start = start // 2 if isinstance(start, int) else pl.multiple_of(start >> 1, align // 2)
        return pltpu.bitcast(view[lead + (pl.ds(start, size // 2), slice(None))], BF16)
    return load


def _dft(freq_axis, shape, first):
    r = lax.broadcasted_iota(I32, shape, freq_axis) + first
    s = lax.broadcasted_iota(I32, shape, 1 - freq_axis)
    m = ((r >> 4) << 3) + (r & 7)
    n = ((4 * m + 1) * s + ((r >> 3) & 1) * 128) & 511
    return jnp.cos(n.astype(F32) * (math.pi / 256.0))


class _Refs:
    def __init__(self, refs):
        self.refs = dict(zip(_SCRATCH, refs))

    def __getattr__(self, name):
        return self.refs[name]


def _body(q_h, k_h, v_h, sk_h, ssm_h, dd_h, wr_h, wg_h, wu_h, wd_h, c_h, wm_h, o_h, R, zero_s, sem_o, sem_i):
    ks, zs = (R.k0, R.k1), (R.z0, R.z1)
    z_ld = (_packed(R.z0), _packed(R.z1))
    kv_ld, n2_ld, fw_ld, iv_ld = (_packed(r) for r in (R.kv, R.n2, R.fw, R.iv))
    ssm_s, wm_s = R.ssm.bitcast(BF16), R.wm.bitcast(BF16)

    def cv_tile(l):
        return pltpu.bitcast(R.cv[:, l * 128:(l + 1) * 128], BF16)

    order = []

    def group(*pairs):
        sem = sem_i.at[len(order)]
        cps = [pltpu.make_async_copy(a, b, sem) for a, b in pairs]
        order.append(cps)
        return cps

    def wait(cps):
        for cp in cps:
            cp.wait()

    def wait_at(i, table):
        for it, cps in table.items():
            @pl.when(i == it)
            def _():
                wait(cps)

    def ssm_group(l):
        rows = pl.ds(l * 128, 128)
        return group((ssm_h.at[rows], ssm_s.at[rows]))

    sk_cp = group((sk_h, R.sk))
    ssm_cps = [ssm_group(0)]
    kv_cps = []
    for c in range(PCH):
        rows = pl.ds(c * (S // PCH), S // PCH)
        kv_cps.append(group((k_h.at[rows], R.k.at[rows]), (v_h.at[rows], R.v.at[rows])))
    small = group((dd_h, R.dd), (wr_h, R.wr), (c_h, R.c))
    ssm_cps += [ssm_group(l) for l in range(1, NT)]
    wm_cp = group((wm_h, wm_s))
    q_cps = []
    for c in range(NQ):
        rows = pl.ds(c * (S // NQ), S // NQ)
        q_cps.append(group((q_h.at[rows], R.q.at[rows])))
    head, tail = pl.ds(0, FF - WD_TAIL), pl.ds(FF - WD_TAIL, WD_TAIL)
    f_head = group((wg_h, R.wg), (wu_h, R.wu), (wd_h.at[head], R.wd.at[head]))
    f_tail = group((wd_h.at[tail], R.wd.at[tail]))
    for cps in order:
        for cp in cps:
            cp.start()

    def o_copy(b):
        rows = pl.ds(pl.multiple_of(b * BLK, BLK), BLK)
        return pltpu.make_async_copy(R.o.at[rows], o_h.at[rows], sem_o)

    R.fw[...] = _dft(0, (256, 128), 0).astype(BF16)
    for h in range(2):
        R.iv[h] = (_dft(1, (128, 128), h * 128) * (1.0 / 128.0)).astype(BF16)
    for l in range(NT):
        R.kf[l, pl.ds(0, 8), :] = jnp.zeros((8, 128), F32)
    for g in range(len(GROUPS)):
        zero_s[g] = 0
    wait(sk_cp)
    skf = R.sk[...].astype(F32)
    for l in range(NT):
        for j in range(4):
            R.tap[l, j] = jnp.broadcast_to(skf[j:j + 1, l * 128:(l + 1) * 128], (8, 128))

    def make_kv(l, t, slot):
        r0 = pl.multiple_of(t * BLK, BLK)
        cols = slice(l * 128, (l + 1) * 128)
        kb = R.k[pl.ds(r0, BLK), cols].astype(F32)
        R.kf[l, pl.ds(r0 + 8, BLK), :] = kb
        w = [jnp.tile(R.tap[l, j], (BLK // 8, 1)) for j in range(4)]
        acc = kb * w[0]
        for j in range(1, 4):
            acc = acc + R.kf[l, pl.ds(r0 + 8 - j, BLK), :] * w[j]
        R.kv[slot] = (acc * R.v[pl.ds(r0, BLK), cols].astype(F32)).astype(BF16)

    def fwd_x(l, t, slot):
        R.x[l, t] = _nn(fw_ld((), 0, 256, 0), kv_ld((slot,), 0, BLK, 0)).reshape(_SPEC[1:])

    def fwd_k(l, t):
        taps = pl.ds(pl.multiple_of(t * BLK, BLK), BLK)
        ks[l % 2][t] = _nt(fw_ld((), 0, 256, 0), ssm_s[l * 128:(l + 1) * 128, taps]).reshape(_SPEC[1:])

    def add_skip(l):
        kk = ks[l % 2]
        kk[0, :, 0] = kk[0, :, 0] + R.dd[l:l + 1, :].astype(F32)

    def wconv(l, t0):
        kk, z = ks[l % 2], zs[l % 2]
        zrows = pl.ds(pl.multiple_of(t0 * 16, 16), 16)
        prev = None
        b0 = 0
        for g, gs in enumerate(GROUPS):
            t = t0 + zero_s[g]
            acc = [None] * gs
            xw = {}
            for j in range(b0 + gs):
                kc, kd = kk[j, t, 0], kk[j, t, 1]
                ke = kc + kd
                for i in range(gs):
                    m = b0 + i - j
                    if m < 0:
                        continue
                    if m not in xw:
                        xa, xb = R.x[l, m, t, 0], R.x[l, m, t, 1]
                        xw[m] = (xa, xb, xa + xb)
                    xa, xb, xu = xw[m]
                    p = (xa * kc, xb * kd, xu * ke)
                    acc[i] = p if acc[i] is None else tuple(u + w for u, w in zip(acc[i], p))
            for i in range(gs):
                s1, s2, s3 = acc[i]
                re, im = s1 - s2, s3 - (s1 + s2)
                if prev is None:
                    zr, zi = re, im
                else:
                    zr, zi = re - prev[1], im + prev[0]
                prev = (re, im)
                z[b0 + i, zrows, :] = jnp.concatenate([zr, zi], axis=0).astype(BF16)
            b0 += gs

    def inv(l, t, ya, yb, rows, g0, n):
        for h, y in enumerate((ya, yb)):
            y[rows, l * 128:(l + 1) * 128] = _nn(iv_ld((h,), g0, n, n), z_ld[l % 2]((t,), h * 128, 128, 0))

    def modchunk(t):
        cols = pl.ds(pl.multiple_of(jnp.minimum(t, 14) * 256, 256), 256)
        for l in range(NT):
            R.mp[l, :, cols] = _nn(cv_tile(l), wm_s[l * 128:(l + 1) * 128, cols])[:8]

    class Win:
        def __init__(self, r0, n):
            rows = pl.ds(r0 if isinstance(r0, int) else pl.multiple_of(r0, RG), n)
            self.q, self.ya, self.yb, self.xx, self.o = (r.at[rows] for r in (R.q, R.ya, R.yb, R.xx, R.o))
            self.st, self.pt, self.n2 = (r.at[:, rows] for r in (R.st, R.pt, R.n2))

    def fold(x):
        acc = x[:, 0:128]
        for l in range(1, NT):
            acc = acc + x[:, l * 128:(l + 1) * 128]
        return acc

    def sums(w, x, rows, slot):
        w.pt[slot, rows, :] = fold(x)
        w.pt[slot + 1, rows, :] = fold(x * x)

    def stage_r(w, r0, n, slot):
        rows = pl.ds(r0, n)
        for j in (slot, slot + 1):
            w.st[j, rows, :] = jnp.broadcast_to(jnp.sum(w.pt[j, rows, :], axis=-1, keepdims=True), (n, 128))

    def stage_a(w, n):
        for s in range(n // SL):
            rows = pl.ds(s * SL, SL)
            sums(w, w.q[rows, :].astype(F32), rows, 0)

    wait(ssm_cps[0])

    def p0(i, _):
        wait_at(i, dict(enumerate(kv_cps)))
        for u in range(PB):
            fwd_k(0, i * PB + u)
        for u in range(PB):
            for l in range(NT):
                make_kv(l, i * PB + u, u * NT + l)
                fwd_x(l, i * PB + u, u * NT + l)
        return 0

    lax.fori_loop(0, PCH, p0, 0)
    wait(small)
    add_skip(0)
    cvec = R.c[...].astype(F32)
    R.cv[...] = pltpu.bitcast(jnp.broadcast_to((cvec * _sigmoid_bf16(cvec)).astype(BF16), (16, D)), U32)

    def p1(i, l):
        last = l + 1 == NT
        if last:
            wait_at(i, {(c * (S // NQ)) // AR: q_cps[c] for c in range(NQ)})
        for u in range(UB):
            if last:
                modchunk(i * UB + u)
            else:
                fwd_k(l + 1, i * UB + u)
        if l >= 1:
            for u in range(UB):
                t = i * UB + u
                inv(l - 1, t, R.ya, R.yb, pl.ds(pl.multiple_of(t * BLK, BLK), BLK), 0, BLK)
        if last:
            stage_r(Win(jnp.maximum(i - 1, 0) * AR, AR), 0, AR, 0)
        for u in range(UB):
            wconv(l, i * UB + u)
        if last:
            stage_a(Win(i * AR, AR), AR)
        return 0

    for l in range(NT):
        if l + 1 < NT:
            wait(ssm_cps[l + 1])
        else:
            wait(wm_cp)
            R.pt[0:2, 0:AR, :] = jnp.zeros((2, AR, 128), F32)
        lax.fori_loop(0, NI, lambda i, _, l=l: p1(i, l), 0)
        if l + 1 < NT:
            add_skip(l + 1)
    stage_r(Win(S - AR, AR), 0, AR, 0)

    md = R.mp[0, 0:1, :]
    for l in range(1, NT):
        md = md + R.mp[l, 0:1, :]
    md = _rb(md)
    sa, ca, ga, sb, cb, gb = (md[:, i * D:(i + 1) * D] for i in range(6))
    ca1, cb1 = _rb(1.0 + ca), _rb(1.0 + cb)
    wr = jnp.concatenate([R.wr[l:l + 1, :] for l in range(NT)], axis=1).astype(F32)
    u_all = cb1 * wr
    u_hi = _rb(u_all)
    rid16 = lax.broadcasted_iota(I32, (16, D), 0)
    R.cv[...] = pltpu.bitcast(
        jnp.where(rid16 == 0, u_hi, jnp.where(rid16 == 1, u_all - u_hi, 0.0)).astype(BF16), U32)
    r_off = jnp.sum(sb * wr, axis=-1, keepdims=True)
    for i, vec in enumerate((ca1 * ga, sa * ga, cb1 * gb, sb * gb)):
        R.cf[i] = jnp.broadcast_to(vec, (8, D))

    def coef(i):
        return jnp.tile(R.cf[i], (SL // 8, 1))

    def wide(a):
        return jnp.tile(a, (1, NT))

    def stats(w, rows, slot):
        m = w.st[slot, rows, :] * (1.0 / D)
        var = jnp.maximum(w.st[slot + 1, rows, :] * (1.0 / D) - m * m, 0.0)
        return m, jnp.exp2(jnp.log(var + EPS) * (-0.5 / math.log(2.0)))

    def slice_b(w, rows, m, rs):
        x = w.q[rows, :].astype(F32)
        x1 = x + (w.ya[rows, :] + w.yb[rows, :]) * ((x - wide(m)) * wide(rs) * coef(0) + coef(1))
        w.xx[rows, :] = x1
        sums(w, x1, rows, 2)

    def slice_c(w, rows, m, rs):
        x1 = w.xx[rows, :]
        n2 = (x1 - wide(m)) * wide(rs)
        for l in range(NT):
            w.n2[l, rows, :] = n2[:, l * 128:(l + 1) * 128].astype(BF16)
        w.o[rows, :] = (x1 + n2 * coef(2) + coef(3)).astype(BF16)

    def stage_bc(w, kb, kc):
        tasks = []
        for fn, k, slot in ((slice_b, kb, 0), (slice_c, kc, 2)):
            if k is not None:
                tasks += [(fn, pl.ds(k * RG + s * SL, SL), slot) for s in range(RG // SL)]
        nxt = stats(w, *tasks[0][1:])
        for i, (fn, rows, _) in enumerate(tasks):
            cur = nxt
            if i + 1 < len(tasks):
                nxt = stats(w, *tasks[i + 1][1:])
            fn(w, rows, *cur)

    def stage_d(g):
        for l in range(NT):
            R.r[l, pl.ds(pl.multiple_of(g * 8, 8), 8), :] = _nt(cv_tile(l), n2_ld((l,), g * RG, RG, RG))[:8]

    def p2_step(g):
        static = isinstance(g, int)
        lo = max(g, 0) if static else g
        n = (min(g + 4, NG) - lo) if static else 4
        w = Win(lo * RG, n * RG) if n > 0 else None
        off = lo - g if static else 0

        def ok(d):
            return (not static) or 0 <= g + d < NG
        if ok(-1):
            stage_d(g - 1)
        if ok(3):
            inv(NT - 1, (g + 3) >> 1, w.ya, w.yb, pl.ds((3 - off) * RG, RG), ((g + 3) & 1) * RG, RG)
        if ok(1):
            stage_r(w, (1 - off) * RG, RG, 2)
        if ok(2) or ok(0):
            stage_bc(w, 2 - off if ok(2) else None, 0 - off if ok(0) else None)
        return 0

    for g in range(-3, 1):
        p2_step(g)
    lax.fori_loop(1, NG - 3, lambda g, _: p2_step(g), 0)
    for g in range(NG - 3, NG + 1):
        p2_step(g)

    r = jnp.broadcast_to(r_off, (NG, RG))
    for l in range(NT):
        r = r + R.r[l, pl.ds(0, NG, stride=8), :] + R.r[l, pl.ds(1, NG, stride=8), :]
    tok = lax.broadcasted_iota(I32, (NG, RG), 0) * RG + lax.broadcasted_iota(I32, (NG, RG), 1)
    r = jnp.clip(jnp.where(jnp.abs(r) < 1e-30, 1e-30, r), -3e38, 3e38)
    bits = lax.bitcast_convert_type(r, I32)
    key = lax.bitcast_convert_type((bits & ~(S - 1)) | jnp.where(bits < 0, tok, S - 1 - tok), F32)

    def amax(x):
        return jnp.max(jnp.max(x, axis=0, keepdims=True), axis=1, keepdims=True)

    def index_of(kv):
        kb = lax.bitcast_convert_type(kv, I32)
        low = kb & (S - 1)
        return jnp.where(kb < 0, low, S - 1 - low)[0, 0]

    m1 = amax(key)
    m2 = amax(jnp.where(key == m1, -jnp.inf, key))
    i1, i2 = index_of(m1), index_of(m2)
    b1, b2 = i1 >> 7, i2 >> 7

    wait(f_head)
    for b in range(NB):
        @pl.when(jnp.logical_and(b != b1, b != b2))
        def _():
            o_copy(b).start(priority=b % 2)

    def grp(i):
        return pl.ds(pl.multiple_of((i >> 4) << 4, 16), 16)

    def two_rows(f):
        return jnp.where(rid16 == 0, f(i1), jnp.where(rid16 == 1, f(i2), 0.0))

    def q_row(i):
        return jnp.sum(jnp.where(rid16 == (i & 15), R.q[grp(i), :].astype(F32), 0.0), axis=0, keepdims=True)

    def ln_rows(x):
        m = jnp.mean(x, axis=-1, keepdims=True)
        var = jnp.mean(jnp.square(x - m), axis=-1, keepdims=True)
        return _rb(_rb(x - _rb(m)) / _rb(jnp.sqrt(_rb(_rb(var) + EPS_BF16))))

    xq = two_rows(q_row)
    yr = _rb(two_rows(lambda i: R.ya[pl.ds(i, 1), :] + R.yb[pl.ds(i, 1), :]))
    hq = _rb(_rb(ln_rows(xq) * ca1) + sa)
    x1r = _rb(xq + _rb(ga * _rb(hq * yr)))
    hr = _rb(_rb(ln_rows(x1r) * cb1) + sb)
    xsel = hr.astype(BF16)
    gate = _rb(_nt(xsel, R.wg[...]))
    up = _rb(_nt(xsel, R.wu[...]))
    act = (_rb(gate * _sigmoid_bf16(gate)) * up).astype(BF16)
    wait(f_tail)
    yf = _rb(_nn(act, R.wd[...]))
    rsel = _sigmoid_bf16(_rb(jnp.where(rid16[:, :1] == 0, m1, m2)))
    fin = x1r + _rb(gb * _rb(hr + _rb(yf * rsel)))
    for row, i in ((0, i1), (1, i2)):
        cur = R.o[grp(i), :].astype(F32)
        R.o[grp(i), :] = jnp.where(rid16 == (i & 15), fin[row:row + 1], cur).astype(BF16)
    o_copy(b1).start()

    @pl.when(b2 != b1)
    def _():
        o_copy(b2).start()


def _kernel(*refs):
    ins, o_h, scr = refs[:12], refs[12], refs[13:]
    R = _Refs(scr)
    zero_s, sem_o = scr[-2], scr[-1]
    pl.run_scoped(lambda sem_i: _body(*ins, o_h, R, zero_s, sem_o, sem_i), pltpu.SemaphoreType.DMA((NSEM,)))
    pltpu.make_async_copy(R.o, o_h, sem_o).wait()


@jax.jit
def pallas_adaLN_cond__ssm_conv_h3__moe_arch_mod__prompt_kernel(
    A_q: jax.Array,
    A_k: jax.Array,
    A_v: jax.Array,
    A_shift_k: jax.Array,
    A_ssm_k: jax.Array,
    A_ssm_D: jax.Array,
    B_x: jax.Array,
    B_w_r: jax.Array,
    B_w_gate: jax.Array,
    B_w_up: jax.Array,
    B_w_down: jax.Array,
    c: jax.Array,
    w_mod: jax.Array,
):
    scratch = [pltpu.VMEM(shape, dt) for shape, dt in _SCRATCH.values()]
    scratch += [pltpu.SMEM((len(GROUPS),), I32), pltpu.SemaphoreType.DMA(())]
    out = pl.pallas_call(
        _kernel,
        out_shape=jax.ShapeDtypeStruct((S, D), BF16),
        in_specs=[pl.BlockSpec(memory_space=pl.ANY)] * 12,
        out_specs=pl.BlockSpec(memory_space=pl.ANY),
        scratch_shapes=scratch,
        compiler_params=pltpu.CompilerParams(vmem_limit_bytes=100 * 1024 * 1024),
    )(A_q.reshape(S, D), A_k.reshape(S, D), A_v.reshape(S, D), A_shift_k.T, A_ssm_k,
      A_ssm_D.reshape(NT, 128), B_w_r.reshape(NT, 128), B_w_gate.T, B_w_up.T, B_w_down, c, w_mod)
    return out.reshape(1, S, D)
```
